```python
import os as _os
_os.environ.setdefault("JAX_PLATFORMS", "cpu")
import jax
import jax.numpy as jnp

def _softmax(x, axis=-1):
    return jax.nn.softmax(x, axis=axis)
def _gelu(x):
    return jax.nn.gelu(x, approximate=True)
def _silu(x):
    return jax.nn.silu(x)
def _sigmoid(x):
    return jax.nn.sigmoid(x)
def _layernorm(x, axis=-1, eps=1e-5):
    m = jnp.mean(x, axis=axis, keepdims=True)
    v = jnp.var(x, axis=axis, keepdims=True)
    return (x - m) / jnp.sqrt(v + eps)
def _scatter_add(tgt, idx, src, axis=0):
    return tgt.at[idx].add(src)
def _segment_sum(src, seg, n):
    return jax.ops.segment_sum(src, seg, n)
class _Rng:
    def __init__(self, key):
        self._k = key
    def _next(self):
        self._k, sub = jax.random.split(self._k)
        return sub
    def normal(self, shape):
        return jax.random.normal(self._next(), shape, dtype=jnp.bfloat16)
    def randint(self, lo, hi, shape):
        return jax.random.randint(self._next(), shape, lo, hi, dtype=jnp.int32)
    def uniform(self, shape, lo=0.0, hi=1.0):
        return jax.random.uniform(self._next(), shape, jnp.bfloat16, lo, hi)
    def permutation(self, n):
        return jax.random.permutation(self._next(), n)


kernel_name = 'concat_heads__mha_block_cached__mha_block_cached__near_ridge'

def setup_inputs():
    _rng = _Rng(jax.random.key(int.from_bytes(__import__("os").urandom(4), "little")))
    _w = (lambda a: (lambda t: t.astype(jnp.bfloat16) if jnp.issubdtype(t.dtype, jnp.floating) else t)(jnp.asarray(a)))
    def _A_setup():
        B, Sq, D = 8, 144, 640
        H, Sk, Dh = 32, 512, 128
        return {
            "x": _w((lambda *s: _rng.normal(s) * 0.8)(B, Sq, D)),
            "k_cache": _w((lambda *s: _rng.normal(s) * 0.8)(B, H, Sk, Dh)),
            "v_cache": _w((lambda *s: _rng.normal(s) * 0.05)(B, H, Sk, Dh)),
            "wq": _w((lambda *s: _rng.normal(s) * 0.8)(D, H * Dh) * (D ** -0.5)),
            "wo": _w((lambda *s: _rng.normal(s) * 0.05)(H * Dh, D) * ((H * Dh) ** -0.5)),
        }
    _A_in = _A_setup()

    def _B_setup():
        B, Sq, D = 8, 144, 640
        H, Sk, Dh = 32, 512, 128
        return {
            "x": _w((lambda *s: _rng.normal(s) * 0.8)(B, Sq, D)),
            "k_cache": _w((lambda *s: _rng.normal(s) * 0.8)(B, H, Sk, Dh)),
            "v_cache": _w((lambda *s: _rng.normal(s) * 0.05)(B, H, Sk, Dh)),
            "wq": _w((lambda *s: _rng.normal(s) * 0.8)(D, H * Dh) * (D ** -0.5)),
            "wo": _w((lambda *s: _rng.normal(s) * 0.05)(H * Dh, D) * ((H * Dh) ** -0.5)),
        }
    _B_in = _B_setup()

    return {
        "A_x": _A_in["x"],
        "A_k_cache": _A_in["k_cache"],
        "A_v_cache": _A_in["v_cache"],
        "A_wq": _A_in["wq"],
        "A_wo": _A_in["wo"],
        "B_x": _B_in["x"],
        "B_k_cache": _B_in["k_cache"],
        "B_v_cache": _B_in["v_cache"],
        "B_wq": _B_in["wq"],
        "B_wo": _B_in["wo"],
    }

def reference(A_x, A_k_cache, A_v_cache, A_wq, A_wo, B_x, B_k_cache, B_v_cache, B_wq, B_wo):
    def _A_ref(x, k_cache, v_cache, wq, wo):
        B, Sq, D = x.shape
        H, Dh = 32, 128
        q = (lambda x, *d: x.transpose(*d))((x @ wq).reshape(B, Sq, H, Dh), 0, 2, 1, 3)
        scores = jnp.einsum("bhqd,bhkd->bhqk", q, k_cache) * (Dh ** -0.5)
        p = _softmax(scores, axis=-1)
        o = jnp.einsum("bhqk,bhkd->bhqd", p, v_cache)
        return (lambda x, *d: x.transpose(*d))(o, 0, 2, 1, 3).reshape(B, Sq, H * Dh) @ wo

    def _B_ref(x, k_cache, v_cache, wq, wo):
        B, Sq, D = x.shape
        H, Dh = 32, 128
        q = (lambda x, *d: x.transpose(*d))((x @ wq).reshape(B, Sq, H, Dh), 0, 2, 1, 3)
        scores = jnp.einsum("bhqd,bhkd->bhqk", q, k_cache) * (Dh ** -0.5)
        p = _softmax(scores, axis=-1)
        o = jnp.einsum("bhqk,bhkd->bhqd", p, v_cache)
        return (lambda x, *d: x.transpose(*d))(o, 0, 2, 1, 3).reshape(B, Sq, H * Dh) @ wo

    a = _A_ref(A_x, A_k_cache, A_v_cache, A_wq, A_wo)
    b = _B_ref(B_x, B_k_cache, B_v_cache, B_wq, B_wo)
    return jnp.concatenate([a, b], axis=-1)
```

```python
import jax, jax.numpy as jnp, numpy as np
import jax.experimental.pallas as pl
import jax.experimental.pallas.tpu as pltpu

B,Sq,D,H,Sk,Dh = 8,144,640,32,512,128
ND = D // 128
LOG2E = 1.4426950408889634
bf = jnp.bfloat16; f32 = jnp.float32; u32 = jnp.uint32
NT = (((1,),(1,)),((),()))

def make_v3(hb=8, nb=2, R=3, vmem=100, qa=2, ka=1, bitc=True, mode="full", op_slots=None, newton=True, qstore=False, inwait=False, nobc=True):
    G = H // hb; NP = 2 * G; IPP = B // nb; NI = NP * IPP
    hpp = hb // IPP
    assert hpp >= 1 and R - 1 <= IPP
    c = (Dh ** -0.5) * LOG2E
    if op_slots is None:
        op_slots = [1 + (n * (hb - 1)) // ND for n in range(ND)]

    def ld(ref):
        if bitc: return pltpu.bitcast(ref.bitcast(u32)[...], bf)
        return ref[...]
    def st(ref, val):
        if bitc: ref.bitcast(u32)[...] = pltpu.bitcast(val, u32)
        else: ref[...] = val

    def kern(ax, ak, av, awq, awo, bx, bk, bv, bwq, bwo, out,
             kbuf, vbuf, wqbuf, wobuf, xbuf, acc, obuf, ostage,
             sk, sv, swq, swo, sx, so):
        X = (ax, bx); K = (ak, bk); V = (av, bv); WQ = (awq, bwq); WO = (awo, bwo)

        def by_branch(br, fn):
            if isinstance(br, int):
                fn(br)
            else:
                pl.when(br == 0)(lambda: fn(0))
                pl.when(br == 1)(lambda: fn(1))

        def k_cp(s, slot, j, b, g):
            return pltpu.make_async_copy(K[s].at[b, pl.ds(g * hb, hb)], kbuf.at[slot, j], sk.at[slot, j])
        def v_cp(s, slot, j, b, g):
            return pltpu.make_async_copy(V[s].at[b, pl.ds(g * hb, hb)], vbuf.at[slot, j], sv.at[slot, j])
        def wq_cp(s, ws, g, h):
            col = pl.multiple_of((g * hb + h) * Dh, Dh)
            return pltpu.make_async_copy(WQ[s].at[:, pl.ds(col, Dh)], wqbuf.at[ws, h], swq.at[ws, h])
        def wo_cp(s, ws, g, h0, nh, n):
            row = pl.multiple_of((g * hb + h0) * Dh, Dh)
            return pltpu.make_async_copy(WO[s].at[pl.ds(row, nh * Dh), pl.ds(n * 128, 128)],
                                         wobuf.at[ws, n, pl.ds(h0 * Dh, nh * Dh)], swo.at[ws, (h0 // hpp) if isinstance(h0, int) else h0 // hpp, n])
        def x_cp(s, b, n):
            return pltpu.make_async_copy(X[s].at[b, :, pl.ds(n * 128, 128)], xbuf.at[s, b, n], sx.at[s, b, n])
        def o_cp(s, b, n):
            return pltpu.make_async_copy(ostage.at[s, b, n], out.at[b, :, pl.ds(s * D + n * 128, 128)], so.at[s, b, n])

        def split(i):
            ph = i // IPP; bb = i % IPP
            return ph, bb, ph // G, ph % G

        def extras(i, act):
            ph, bb, br, g = split(i)
            ph1 = ph + 1
            def wpart(s):
                g1 = ph1 % G; ws = ph1 % 3
                for t in range(hpp):
                    getattr(wq_cp(s, ws, g1, bb * hpp + t), act)()
                for n in range(ND):
                    getattr(wo_cp(s, ws, g1, bb * hpp, hpp, n), act)()
            def xpart(s):
                bb1 = (i + 1) % IPP
                for j in range(nb):
                    for n in range(ND):
                        getattr(x_cp(s, bb1 * nb + j, n), act)()
            i1 = i + 1
            if isinstance(i, int):
                if i1 < NI and (i1 // IPP) % G == 0: xpart(i1 // IPP // G)
                if ph1 < NP: wpart(ph1 // G)
            else:
                @pl.when(jnp.logical_and(i1 < NI, (i1 // IPP) % G == 0))
                def _():
                    by_branch(i1 // IPP // G, xpart)
                @pl.when(ph1 < NP)
                def _():
                    by_branch(ph1 // G, wpart)

        def issue_kv(i):
            ph, bb, br, g = split(i); slot = i % R
            def f(s):
                for j in range(nb):
                    k_cp(s, slot, j, bb * nb + j, g).start()
                    v_cp(s, slot, j, bb * nb + j, g).start()
            by_branch(br, f)

        for j in range(nb):
            for n in range(ND): x_cp(0, j, n).start()
            if j == 0:
                for h in range(hb): wq_cp(0, 0, 0, h).start()
            k_cp(0, 0, j, j, 0).start(); v_cp(0, 0, j, j, 0).start()
            if j == 0:
                for bbx in range(IPP):
                    for n in range(ND): wo_cp(0, 0, 0, bbx * hpp, hpp, n).start()
        extras(0, "start")
        for i0 in range(1, R - 1):
            issue_kv(i0); extras(i0, "start")
        acc[...] = jnp.zeros(acc.shape, f32)
        for j in range(nb):
            for n in range(ND): x_cp(0, j, n).wait()
        for h in range(hb): wq_cp(0, 0, 0, h).wait()
        for bbx in range(IPP):
            for n in range(ND): wo_cp(0, 0, 0, bbx * hpp, hpp, n).wait()

        def body(i, carry):
            ph, bb, br, g = split(i); slot = i % R; ws = ph % 3
            @pl.when(i + R - 1 < NI)
            def _():
                issue_kv(i + R - 1); extras(i + R - 1, "start")
            @pl.when(i >= 1)
            def _():
                extras(i - 1, "wait")
            if mode == "dma" or not inwait:
                for j in range(nb):
                    k_cp(0, slot, j, 0, 0).wait(); v_cp(0, slot, j, 0, 0).wait()
            if mode != "dma":
                compute(i, bb, br, slot, ws)
            @pl.when(g == G - 1)
            def _():
                def f(s):
                    for j in range(nb):
                        for n in range(ND): o_cp(s, bb * nb + j, n).start()
                by_branch(br, f)
            return carry

        def compute(i, bb, br, slot, ws):
            n_units = nb * hb
            q = {}; s = {}; p = {}; l = {}
            xv = {}
            def getx(j):
                b = bb * nb + j
                return jnp.concatenate([ld(xbuf.at[br, b, n]) for n in range(ND)], axis=1)
            def QP(u):
                j, h = divmod(u, hb)
                r = jnp.dot(getx(j), ld(wqbuf.at[ws, h]), preferred_element_type=f32)
                q[u] = (r * c).astype(bf)
            def QK(u):
                j, h = divmod(u, hb)
                if h == 0 and inwait: k_cp(0, slot, j, 0, 0).wait()
                s[u] = jax.lax.dot_general(q.pop(u), ld(kbuf.at[slot, j, h]), NT, preferred_element_type=f32)
            def SM(u):
                su = s.pop(u)
                m = jnp.max(su, axis=-1, keepdims=True)
                e = jnp.exp2(su - m)
                l[u] = jnp.sum(e, axis=-1, keepdims=True)
                p[u] = e.astype(bf)
            def PV(u):
                j, h = divmod(u, hb)
                if h == 0 and inwait: v_cp(0, slot, j, 0, 0).wait()
                r = jnp.dot(p.pop(u), ld(vbuf.at[slot, j, h]), preferred_element_type=f32)
                lu = l.pop(u)
                if newton:
                    r0 = pl.reciprocal(lu, approx=True)
                    inv = r0 * (2.0 - lu * r0)
                else:
                    inv = 1.0 / lu
                st(obuf.at[j, h], (r * inv).astype(bf))
            def OP(j, n):
                b = bb * nb + j
                oo = jnp.concatenate([ld(obuf.at[j, h]) for h in range(hb)], axis=1)
                r = jnp.dot(oo, ld(wobuf.at[ws, n]), preferred_element_type=f32)
                r = r + acc[br, b, :, n * 128:(n + 1) * 128]
                acc[br, b, :, n * 128:(n + 1) * 128] = r
                st(ostage.at[br, b, n], r.astype(bf))
            for t in range(-qa, n_units):
                if t + qa < n_units: QP(t + qa)
                if 0 <= t + ka < n_units: QK(t + ka)
                if t >= 0:
                    j, h = divmod(t, hb)
                    if j >= 1:
                        for n in range(ND):
                            if op_slots[n] == h: OP(j - 1, n)
                    SM(t); PV(t)
            for n in range(ND): OP(nb - 1, n)

        jax.lax.fori_loop(0, NI, body, 0)
        for s in range(2):
            for b in range(B):
                for n in range(ND): o_cp(s, b, n).wait()

    ANY = pl.BlockSpec(memory_space=pl.ANY)
    def f(ax, ak, av, awq, awo, bx, bk, bv, bwq, bwo):
        return pl.pallas_call(
            kern, in_specs=[ANY]*10, out_specs=ANY,
            out_shape=jax.ShapeDtypeStruct((B,Sq,2*D), bf),
            scratch_shapes=[
                pltpu.VMEM((R, nb, hb, Sk, Dh), bf), pltpu.VMEM((R, nb, hb, Sk, Dh), bf),
                pltpu.VMEM((3, hb, D, Dh), bf), pltpu.VMEM((3, ND, hb*Dh, 128), bf),
                pltpu.VMEM((2, B, ND, Sq, 128), bf), pltpu.VMEM((2, B, Sq, D), f32),
                pltpu.VMEM((nb, hb, Sq, Dh), bf), pltpu.VMEM((2, B, ND, Sq, 128), bf),
                pltpu.SemaphoreType.DMA((R, nb)), pltpu.SemaphoreType.DMA((R, nb)),
                pltpu.SemaphoreType.DMA((3, hb)), pltpu.SemaphoreType.DMA((3, IPP, ND)),
                pltpu.SemaphoreType.DMA((2, B, ND)), pltpu.SemaphoreType.DMA((2, B, ND)),
            ],
            compiler_params=pltpu.CompilerParams(vmem_limit_bytes=vmem*1024*1024, disable_bounds_checks=nobc),
        )(ax, ak, av, awq, awo, bx, bk, bv, bwq, bwo)
    return f


_kernel_impl = make_v3(nb=2)


@jax.jit
def pallas_concat_heads__mha_block_cached__mha_block_cached__near_ridge_kernel(
    A_x: jax.Array,
    A_k_cache: jax.Array,
    A_v_cache: jax.Array,
    A_wq: jax.Array,
    A_wo: jax.Array,
    B_x: jax.Array,
    B_k_cache: jax.Array,
    B_v_cache: jax.Array,
    B_wq: jax.Array,
    B_wo: jax.Array,
):
    return _kernel_impl(A_x, A_k_cache, A_v_cache, A_wq, A_wo, B_x, B_k_cache, B_v_cache, B_wq, B_wo)
```

```python
import jax, jax.numpy as jnp, numpy as np
from jax import lax
import jax.experimental.pallas as pl
import jax.experimental.pallas.tpu as pltpu

B,Sq,D,H,Sk,Dh = 8,144,640,32,512,128
ND = D // 128
LOG2E = 1.4426950408889634
bf = jnp.bfloat16; f32 = jnp.float32; u32 = jnp.uint32
NT = (((1,),(1,)),((),()))
FL = {"rdd": {"XLA_TPU_RESCHEDULE_DMA_DONES": True}, "lp": {"XLA_TPU_FORCE_LP_LLO_SCHEDULER": True},
      "edc": {"XLA_TPU_EVENLY_DISTRIBUTE_CRITICAL_NODES": True}, "slf": {"XLA_TPU_ENABLE_LLO_SMALL_LOOP_FLATTENING": True},
      "mip": {"XLA_TPU_MAX_INSTS_TO_PREDICATE": 65536}}

def make_v4(hb=4, vmem=100, qa=2, ka=1, mode="full", op_slots=None, flags="rdd", kch=None, PD=8, anchor=False, scope=False):
    G = H // hb; NP = 2 * G
    assert B <= PD <= 2 * B
    kch = kch or hb
    NC = hb // kch
    c = (Dh ** -0.5) * LOG2E
    if op_slots is None:
        op_slots = [(n * hb) // ND for n in range(ND)]
        if op_slots[0] == 0 and hb >= 8: op_slots = [1 + (n * (hb - 1)) // ND for n in range(ND)]
    fl = {}
    if flags:
        for nm in flags.split("+"): fl.update(FL[nm])

    def ld(ref): return pltpu.bitcast(ref.bitcast(u32)[...], bf)
    def st(ref, val): ref.bitcast(u32)[...] = pltpu.bitcast(val, u32)

    def kern(ax, ak, av, awq, awo, bx, bk, bv, bwq, bwo, out,
             kbuf, vbuf, wqbuf, wobuf, xbuf, acc, obuf, ostage,
             sk, sv, swq, swo, sx, so):
        X = (ax, bx); K = (ak, bk); V = (av, bv); WQ = (awq, bwq); WO = (awo, bwo)

        class _Nop:
            def start(self): pass
            def wait(self): pass
        class _NoWait:
            def __init__(self, c): self.c = c
            def start(self): self.c.start()
            def wait(self): pass
        def mk(*a):
            if mode == "comp": return _Nop()
            if mode == "nowait": return _NoWait(pltpu.make_async_copy(*a))
            return pltpu.make_async_copy(*a)
        def arms(pred, br, fn):
            if isinstance(br, int):
                if pred: fn(br)
            else:
                pl.when(jnp.logical_and(pred, br == 0))(lambda: fn(0))
                pl.when(jnp.logical_and(pred, br == 1))(lambda: fn(1))

        def k_cp(s, slot, j, cc, g):
            return mk(K[s].at[j, pl.ds(g * hb + cc * kch, kch)], kbuf.at[slot, j, pl.ds(cc * kch, kch)], sk.at[slot, j, cc])
        def v_cp(s, slot, j, cc, g):
            return mk(V[s].at[j, pl.ds(g * hb + cc * kch, kch)], vbuf.at[slot, j, pl.ds(cc * kch, kch)], sv.at[slot, j, cc])
        def wq_cp(s, ws, g, h):
            col = pl.multiple_of((g * hb + h) * Dh, Dh)
            return mk(WQ[s].at[:, pl.ds(col, Dh)], wqbuf.at[ws, h], sk.at[2, ws, ND + h] if anchor else swq.at[ws, h])
        def wo_cp(s, ws, g, n):
            row = pl.multiple_of(g * hb * Dh, hb * Dh)
            return mk(WO[s].at[pl.ds(row, hb * Dh), pl.ds(n * 128, 128)], wobuf.at[ws, n], sk.at[2, ws, n] if anchor else swo.at[ws, n])
        def x_cp(s, pr, n):
            return mk(X[s].at[pl.ds(2 * pr, 2), :, pl.ds(pl.multiple_of(n * 128, 128), 128)], xbuf.at[s, n, pl.ds(2 * pr, 2)], sx.at[s, pr])
        def x_wait(s, pr):
            mk(xbuf.at[s, :, pl.ds(2 * pr, 2)], xbuf.at[s, :, pl.ds(2 * pr, 2)], sx.at[s, pr]).wait()
        def o_cp(s, b, n):
            col = pl.multiple_of(s * D + n * 128, 128)
            return mk(ostage.at[s, b, n], out.at[b, :, pl.ds(col, 128)], so.at[s, b, n])

        def req_wq(i, h):
            arms(i < NP, i // G, lambda s: wq_cp(s, i % 3, i % G, h).start())
        def req_wo(i, n):
            arms(i < NP, i // G, lambda s: wo_cp(s, i % 3, i % G, n).start())
        def req_k(i, j):
            def f(s):
                for cc in range(NC): k_cp(s, i % 2, j, cc, i % G).start()
            arms(i < NP, i // G, f)
        def req_v(i, j):
            def f(s):
                for cc in range(NC): v_cp(s, i % 2, j, cc, i % G).start()
            arms(i < NP, i // G, f)
        def req_x(i, j):
            if j % 2: return
            def f(s):
                for n in range(ND): x_cp(s, j // 2, n).start()
            if isinstance(i, int):
                if i % G == 0 and i < NP: f(i // G)
            else:
                pl.when(i == G)(lambda: f(1))
        def target(i, j):
            return i + (j + PD) // B, (j + PD) % B
        NPv = NP
        def fence(name, i, fn):
            fn()
        def req_before_k(i, j):
            fence("rx", i, lambda: req_x(i, j))
            if j == 0:
                for h in range(hb): fence("rq", i, lambda: req_wq(i, h))
            fence("rk", i, lambda: req_k(i, j))
        def req_after_v(i, j):
            fence("rv", i, lambda: req_v(i, j))
            if j == 0:
                for n in range(ND): fence("ro", i, lambda: req_wo(i, n))

        import contextlib
        def loop(n, fn):
            def bd(t, c):
                fn(t); return c
            lax.fori_loop(0, n, bd, 0)
        with (jax.named_scope("pro") if scope else contextlib.nullcontext()):
            assert PD == B
            loop(ND, lambda n: x_cp(0, 0, n).start())
            loop(hb, lambda h: wq_cp(0, 0, 0, h).start())
            def first(j):
                @pl.when(j == 1)
                def _():
                    for n in range(ND): wo_cp(0, 0, 0, n).start()
                for cc in range(NC): k_cp(0, 0, j, cc, 0).start()
                for cc in range(NC): v_cp(0, 0, j, cc, 0).start()
                @pl.when(jnp.logical_and(j % 2 == 1, j < B - 1))
                def _():
                    for n in range(ND): x_cp(0, (j + 1) // 2, n).start()
            loop(B, first)
            acc[...] = jnp.zeros(acc.shape, f32)

        def body(i, carry):
            g = lax.rem(i, G); br = lax.div(i, G)
            slot = lax.rem(i, 2); ws = lax.rem(i, 3)
            i2 = i + 2
            n_units = B * hb
            q = {}; s = {}; p = {}; l = {}
            do = mode != "dma"
            def getx(j):
                return jnp.concatenate([ld(xbuf.at[br, n, j]) for n in range(ND)], axis=1)
            def QP(u):
                j, h = divmod(u, hb)
                if h == 0 and j % 2 == 0:
                    pl.when(g == 0)(lambda: x_wait(br, j // 2))
                if j == 0:
                    wq_cp(0, ws, 0, h).wait()
                if not do: return
                r = jnp.dot(getx(j), ld(wqbuf.at[ws, h]), preferred_element_type=f32)
                q[u] = (r * c).astype(bf)
            def QK(u):
                j, h = divmod(u, hb)
                if h % kch == 0: k_cp(0, slot, j, h // kch, 0).wait()
                if do:
                    s[u] = lax.dot_general(q.pop(u), ld(kbuf.at[slot, j, h]), NT, preferred_element_type=f32)
                if h == hb - 1:
                    req_before_k(*target(i, j))
            def SM(u):
                if not do: return
                su = s.pop(u)
                m = jnp.max(su, axis=-1, keepdims=True)
                e = jnp.exp2(su - m)
                l[u] = jnp.sum(e, axis=-1, keepdims=True)
                p[u] = e.astype(bf)
            def PV(u):
                j, h = divmod(u, hb)
                if h % kch == 0: v_cp(0, slot, j, h // kch, 0).wait()
                if do:
                    r = jnp.dot(p.pop(u), ld(vbuf.at[slot, j, h]), preferred_element_type=f32)
                    lu = l.pop(u)
                    r0 = pl.reciprocal(lu, approx=True)
                    inv = r0 * (2.0 - lu * r0)
                    st(obuf.at[j % 2, h], (r * inv).astype(bf))
                if h == hb - 1:
                    req_after_v(*target(i, j))
            def OP(j, n):
                if j == 0:
                    wo_cp(0, ws, 0, n).wait()
                if do:
                    oo = jnp.concatenate([ld(obuf.at[j % 2, h]) for h in range(hb)], axis=1)
                    r = jnp.dot(oo, ld(wobuf.at[ws, n]), preferred_element_type=f32)
                    r = r + acc[br, j, :, n * 128:(n + 1) * 128]
                    acc[br, j, :, n * 128:(n + 1) * 128] = r
                    st(ostage.at[br, j, n], r.astype(bf))
                pl.when(g == G - 1)(lambda: o_cp(br, j, n).start())
            import contextlib
            def step(t):
                if t + qa < n_units: QP(t + qa)
                if 0 <= t + ka < n_units: QK(t + ka)
                if t >= 0:
                    j, h = divmod(t, hb)
                    if j >= 1:
                        for n in range(ND):
                            if op_slots[n] == h: OP(j - 1, n)
                    SM(t); PV(t)
            for t in range(-qa, 0):
                with (jax.named_scope(f"pre{t+qa}") if scope == 2 else contextlib.nullcontext()):
                    step(t)
            for j in range(B):
                with (jax.named_scope(f"g{j}") if scope == 2 else contextlib.nullcontext()):
                    for h in range(hb): step(j * hb + h)
            for n in range(ND): OP(B - 1, n)
            return carry

        def body_s(i, c):
            with jax.named_scope("it"):
                return body(i, c)
        lax.fori_loop(0, NP, body_s if scope else body, 0)
        if mode == "nowait":
            W = lambda c: c.c.wait()
            for i0 in range(NP):
                for h in range(hb): W(wq_cp(0, i0 % 3, 0, h))
                for n in range(ND): W(wo_cp(0, i0 % 3, 0, n))
                for j in range(B):
                    for cc in range(NC):
                        W(k_cp(0, i0 % 2, j, cc, 0)); W(v_cp(0, i0 % 2, j, cc, 0))
            for s in range(2):
                for b in range(B):
                    if b % 2 == 0: x_cp(s, b // 2, 0).c.wait if False else pltpu.make_async_copy(xbuf.at[s, :, pl.ds(b, 2)], xbuf.at[s, :, pl.ds(b, 2)], sx.at[s, b // 2]).wait()
                    for n in range(ND): W(o_cp(s, b, n))
        for s in range(2):
            for b in range(B):
                for n in range(ND): o_cp(s, b, n).wait()

    ANY = pl.BlockSpec(memory_space=pl.ANY)
    def f(ax, ak, av, awq, awo, bx, bk, bv, bwq, bwo):
        return pl.pallas_call(
            kern, in_specs=[ANY]*10, out_specs=ANY,
            out_shape=jax.ShapeDtypeStruct((B,Sq,2*D), bf),
            scratch_shapes=[
                pltpu.VMEM((2, B, hb, Sk, Dh), bf), pltpu.VMEM((2, B, hb, Sk, Dh), bf),
                pltpu.VMEM((3, hb, D, Dh), bf), pltpu.VMEM((3, ND, hb*Dh, 128), bf),
                pltpu.VMEM((2, ND, B, Sq, 128), bf), pltpu.VMEM((2, B, Sq, D), f32),
                pltpu.VMEM((2, hb, Sq, Dh), bf), pltpu.VMEM((2, B, ND, Sq, 128), bf),
                pltpu.SemaphoreType.DMA((3, B, max(NC, ND + hb))), pltpu.SemaphoreType.DMA((2, B, NC)),
                pltpu.SemaphoreType.DMA((3, hb)), pltpu.SemaphoreType.DMA((3, ND)),
                pltpu.SemaphoreType.DMA((2, B // 2)), pltpu.SemaphoreType.DMA((2, B, ND)),
            ],
            compiler_params=pltpu.CompilerParams(vmem_limit_bytes=vmem*1024*1024, disable_bounds_checks=True, flags=fl or None),
        )(ax, ak, av, awq, awo, bx, bk, bv, bwq, bwo)
    return f


_kernel_impl = make_v4(hb=4, PD=8, qa=3, ka=2)


@jax.jit
def pallas_concat_heads__mha_block_cached__mha_block_cached__near_ridge_kernel(
    A_x: jax.Array,
    A_k_cache: jax.Array,
    A_v_cache: jax.Array,
    A_wq: jax.Array,
    A_wo: jax.Array,
    B_x: jax.Array,
    B_k_cache: jax.Array,
    B_v_cache: jax.Array,
    B_wq: jax.Array,
    B_wo: jax.Array,
):
    return _kernel_impl(A_x, A_k_cache, A_v_cache, A_wq, A_wo, B_x, B_k_cache, B_v_cache, B_wq, B_wo)
```

```python
import jax
import jax.numpy as jnp
from jax import lax
import jax.experimental.pallas as pl
import jax.experimental.pallas.tpu as pltpu

_B, _SQ, _D = 8, 144, 640
_H, _SK, _DH = 32, 512, 128
_HB = 4
_G = _H // _HB
_LG = 3
_NP = 2 * _G
_ND = _D // 128
_OP_SLOT = (0, 0, 1, 1, 2)
_XB_AT = 5
_QSCALE = (_DH ** -0.5) * 1.4426950408889634
_NT = (((1,), (1,)), ((), ()))


def _load(ref):
    return pltpu.bitcast(ref.bitcast(jnp.uint32)[...], jnp.bfloat16)


def _store(ref, val):
    ref.bitcast(jnp.uint32)[...] = pltpu.bitcast(val, jnp.uint32)


def _loop(lo, hi, fn):
    def step(t, carry):
        fn(t)
        return carry
    lax.fori_loop(lo, hi, step, 0)


def _kernel(ax, ak, av, awq, awo, bx, bk, bv, bwq, bwo, out,
            kvbuf, wqbuf, wobuf, xbuf, acc, obuf, ostage, skv, swo, sx, so):
    f32, bf16 = jnp.float32, jnp.bfloat16
    x_hbm, wq_hbm, wo_hbm = (ax, bx), (awq, bwq), (awo, bwo)
    kv_hbm = ((ak, bk), (av, bv))

    def wait(dst, sem):
        pltpu.make_async_copy(dst, dst, sem).wait()

    def for_branch(pred, br, fn):
        pl.when(jnp.logical_and(pred, br == 0))(lambda: fn(0))
        pl.when(jnp.logical_and(pred, br == 1))(lambda: fn(1))

    def start_kv(s, w, slot, j, g):
        pltpu.make_async_copy(kv_hbm[w][s].at[j, pl.ds(g * _HB, _HB)],
                              kvbuf.at[slot, j, w], skv.at[slot, j, w]).start()

    def start_wq(s, ws, g, h):
        col = pl.multiple_of((g * _HB + h) * _DH, _DH)
        pltpu.make_async_copy(wq_hbm[s].at[:, pl.ds(col, _DH)],
                              wqbuf.at[ws, h], skv.at[2, ws, 0]).start()

    def start_wo(s, ws, g, n):
        row = pl.multiple_of(g * (_HB * _DH), _HB * _DH)
        pltpu.make_async_copy(wo_hbm[s].at[pl.ds(row, _HB * _DH), pl.ds(n * 128, 128)],
                              wobuf.at[ws, n], swo.at[ws]).start()

    def start_x(s, pair, n):
        col = pl.multiple_of(n * 128, 128)
        pltpu.make_async_copy(x_hbm[s].at[pl.ds(2 * pair, 2), :, pl.ds(col, 128)],
                              xbuf.at[s, n, pl.ds(2 * pair, 2)], sx.at[s, pair]).start()

    _loop(0, _ND, lambda n: start_x(0, 0, n))
    _loop(0, _HB, lambda h: start_wq(0, 0, 0, h))

    def request_x_pair(pair):
        for n in range(_ND):
            start_x(0, pair, n)
    _loop(1, _B // 2, request_x_pair)

    def request_first_kv(j):
        @pl.when(j == 1)
        def _():
            for n in range(_ND):
                start_wo(0, 0, 0, n)
        start_kv(0, 0, 0, j, 0)
        start_kv(0, 1, 0, j, 0)
    _loop(0, _B, request_first_kv)

    acc[...] = jnp.zeros(acc.shape, f32)

    def phase(i, ws):
        ws1 = jnp.where(ws == 2, 0, ws + 1)
        g, br, slot = i & (_G - 1), i >> _LG, i & 1
        i1 = i + 1
        g1, br1, slot1 = i1 & (_G - 1), i1 >> _LG, i1 & 1
        more = i1 < _NP
        units = _B * _HB
        q, scores = {}, {}

        def q_proj(u):
            j, h = divmod(u, _HB)
            if h == 0 and j % 2 == 0:
                pl.when(g == 0)(lambda: wait(xbuf.at[br, :, pl.ds(j, 2)], sx.at[br, j // 2]))
            if u == 0:
                wait(wqbuf.at[ws], skv.at[2, ws, 0])
            x = jnp.concatenate([_load(xbuf.at[br, n, j]) for n in range(_ND)], axis=1)
            r = jnp.dot(x, _load(wqbuf.at[ws, h]), preferred_element_type=f32)
            q[u] = (r * _QSCALE).astype(bf16)

        def qk(u):
            j, h = divmod(u, _HB)
            if h == 0:
                wait(kvbuf.at[slot, j, 0], skv.at[slot, j, 0])
            scores[u] = lax.dot_general(q[u], _load(kvbuf.at[slot, j, 0, h]), _NT,
                                        preferred_element_type=f32)
            if h == _HB - 1:
                if j % 2 == 0:
                    @pl.when(i1 == _XB_AT)
                    def _():
                        for n in range(_ND):
                            start_x(1, j // 2, n)
                if j == 0:
                    for hh in range(_HB):
                        for_branch(more, br1, lambda s: start_wq(s, ws1, g1, hh))
                for_branch(more, br1, lambda s: start_kv(s, 0, slot1, j, g1))

        def softmax_pv(u):
            j, h = divmod(u, _HB)
            s = scores[u]
            e = jnp.exp2(s - jnp.max(s, axis=-1, keepdims=True))
            denom = jnp.sum(e, axis=-1, keepdims=True)
            if h == 0:
                wait(kvbuf.at[slot, j, 1], skv.at[slot, j, 1])
            r = jnp.dot(e.astype(bf16), _load(kvbuf.at[slot, j, 1, h]), preferred_element_type=f32)
            r0 = pl.reciprocal(denom, approx=True)
            inv = r0 * (2.0 - denom * r0)
            _store(obuf.at[j % 2, h], (r * inv).astype(bf16))
            if h == _HB - 1:
                for_branch(more, br1, lambda s_: start_kv(s_, 1, slot1, j, g1))
                if j == 0:
                    for n in range(_ND):
                        for_branch(more, br1, lambda s_: start_wo(s_, ws1, g1, n))

        def out_proj(j, n):
            if j == 0 and n == 0:
                wait(wobuf.at[ws], swo.at[ws])
            o = jnp.concatenate([_load(obuf.at[j % 2, h]) for h in range(_HB)], axis=1)
            r = jnp.dot(o, _load(wobuf.at[ws, n]), preferred_element_type=f32)
            cols = slice(n * 128, (n + 1) * 128)
            r = r + acc[br, j, :, cols]
            acc[br, j, :, cols] = r
            _store(ostage.at[br, j, n], r.astype(bf16))

            @pl.when(g == _G - 1)
            def _():
                col = pl.multiple_of(br * _D + n * 128, 128)
                pltpu.make_async_copy(ostage.at[br, j, n], out.at[j, :, pl.ds(col, 128)],
                                      so.at[0]).start()

        for u in range(units):
            q_proj(u)
        for t in range(-1, units):
            if t + 1 < units:
                qk(t + 1)
            if t >= 0:
                j, h = divmod(t, _HB)
                if j >= 1:
                    for n in range(_ND):
                        if _OP_SLOT[n] == h:
                            out_proj(j - 1, n)
                softmax_pv(t)
        for n in range(_ND):
            out_proj(_B - 1, n)
        return ws1

    lax.fori_loop(0, _NP, phase, jnp.int32(0), unroll=2)
    wait(ostage, so.at[0])


@jax.jit
def pallas_concat_heads__mha_block_cached__mha_block_cached__near_ridge_kernel(
    A_x: jax.Array,
    A_k_cache: jax.Array,
    A_v_cache: jax.Array,
    A_wq: jax.Array,
    A_wo: jax.Array,
    B_x: jax.Array,
    B_k_cache: jax.Array,
    B_v_cache: jax.Array,
    B_wq: jax.Array,
    B_wo: jax.Array,
):
    bf16 = jnp.bfloat16
    hbm = pl.BlockSpec(memory_space=pl.ANY)
    dma = pltpu.SemaphoreType.DMA
    return pl.pallas_call(
        _kernel,
        in_specs=[hbm] * 10,
        out_specs=hbm,
        out_shape=jax.ShapeDtypeStruct((_B, _SQ, 2 * _D), bf16),
        scratch_shapes=[
            pltpu.VMEM((2, _B, 2, _HB, _SK, _DH), bf16),
            pltpu.VMEM((3, _HB, _D, _DH), bf16),
            pltpu.VMEM((3, _ND, _HB * _DH, 128), bf16),
            pltpu.VMEM((2, _ND, _B, _SQ, 128), bf16),
            pltpu.VMEM((2, _B, _SQ, _D), jnp.float32),
            pltpu.VMEM((2, _HB, _SQ, _DH), bf16),
            pltpu.VMEM((2, _B, _ND, _SQ, 128), bf16),
            dma((3, _B, 2)), dma((3,)), dma((2, _B // 2)), dma((1,)),
        ],
        compiler_params=pltpu.CompilerParams(
            vmem_limit_bytes=100 * 1024 * 1024,
            disable_bounds_checks=True,
            disable_semaphore_checks=True,
            flags={"XLA_TPU_RESCHEDULE_DMA_DONES": True},
        ),
    )(A_x, A_k_cache, A_v_cache, A_wq, A_wo, B_x, B_k_cache, B_v_cache, B_wq, B_wo)
```

```python
import jax
import jax.numpy as jnp
from jax import lax
import jax.experimental.pallas as pl
import jax.experimental.pallas.tpu as pltpu

_B, _SQ, _D = 8, 144, 640
_H, _SK, _DH = 32, 512, 128
_HB = 4
_G = _H // _HB
_LG = 3
_NP = 2 * _G
_ND = _D // 128
_OP_SLOT = (0, 1, 2, 3, 3)
_CHUNKS = (1, 1, 1, 1, 2, 2, 2, 2)
_NPLAIN = 4
_MC = 2
_XB_AT = 5
_QSCALE = (_DH ** -0.5) * 1.4426950408889634
_NT = (((1,), (1,)), ((), ()))


def _load(ref):
    return pltpu.bitcast(ref.bitcast(jnp.uint32)[...], jnp.bfloat16)


def _loop(lo, hi, fn):
    def step(t, carry):
        fn(t)
        return carry
    lax.fori_loop(lo, hi, step, 0)


def _kernel(ax, ak, av, awq, awo, bx, bk, bv, bwq, bwo, out,
            kvbuf, wqbuf, wobuf, xbuf, acc, obuf, ostage, skv, swo, sx, so):
    f32, bf16 = jnp.float32, jnp.bfloat16
    x_hbm, wq_hbm, wo_hbm = (ax, bx), (awq, bwq), (awo, bwo)
    kv_hbm = ((ak, bk), (av, bv))

    def wait(dst, sem):
        pltpu.make_async_copy(dst, dst, sem).wait()

    def for_branch(pred, br, fn):
        pl.when(jnp.logical_and(pred, br == 0))(lambda: fn(0))
        pl.when(jnp.logical_and(pred, br == 1))(lambda: fn(1))

    def kv_part(w, slot, j, c, chunks):
        n = _HB // chunks
        return kvbuf.at[slot, j, w, pl.ds(c * n, n)], skv.at[slot, j, w * _MC + c]

    def start_kv(s, w, slot, j, g, c=0, chunks=1):
        n = _HB // chunks
        pltpu.make_async_copy(kv_hbm[w][s].at[j, pl.ds(g * _HB + c * n, n)],
                              *kv_part(w, slot, j, c, chunks)).start()

    def start_wq(s, ws, g, h):
        col = pl.multiple_of((g * _HB + h) * _DH, _DH)
        pltpu.make_async_copy(wq_hbm[s].at[:, pl.ds(col, _DH)],
                              wqbuf.at[ws, h], skv.at[2, ws, 0]).start()

    def start_wo(s, ws, g, n):
        row = pl.multiple_of(g * (_HB * _DH), _HB * _DH)
        pltpu.make_async_copy(wo_hbm[s].at[pl.ds(row, _HB * _DH), pl.ds(n * 128, 128)],
                              wobuf.at[ws, n], swo.at[ws]).start()

    def start_x(s, pair, n):
        col = pl.multiple_of(n * 128, 128)
        pltpu.make_async_copy(x_hbm[s].at[pl.ds(2 * pair, 2), :, pl.ds(col, 128)],
                              xbuf.at[s, n, pl.ds(2 * pair, 2)], sx.at[s, pair]).start()

    _loop(0, _ND, lambda n: start_x(0, 0, n))
    _loop(0, _HB, lambda h: start_wq(0, 0, 0, h))

    def request_x_pair(pair):
        for n in range(_ND):
            start_x(0, pair, n)
    _loop(1, _B // 2, request_x_pair)

    def request_first_kv(j):
        @pl.when(j == 1)
        def _():
            for n in range(_ND):
                start_wo(0, 0, 0, n)
        start_kv(0, 0, 0, j, 0)
        start_kv(0, 1, 0, j, 0)
    _loop(0, _NPLAIN, request_first_kv)
    for j in range(_NPLAIN, _B):
        for c in range(_CHUNKS[j]):
            start_kv(0, 0, 0, j, 0, c, _CHUNKS[j])
            start_kv(0, 1, 0, j, 0, c, _CHUNKS[j])

    acc[...] = jnp.zeros(acc.shape, f32)

    def phase(i, ws):
        ws1 = jnp.where(ws == 2, 0, ws + 1)
        g, br, slot = i & (_G - 1), i >> _LG, i & 1
        i1 = i + 1
        g1, br1, slot1 = i1 & (_G - 1), i1 >> _LG, i1 & 1
        more = i1 < _NP
        units = _B * _HB
        q, scores = {}, {}

        def q_proj(u):
            j, h = divmod(u, _HB)
            if h == 0 and j % 2 == 0:
                pl.when(g == 0)(lambda: wait(xbuf.at[br, :, pl.ds(j, 2)], sx.at[br, j // 2]))
            if u == 0:
                wait(wqbuf.at[ws], skv.at[2, ws, 0])
            x = jnp.concatenate([_load(xbuf.at[br, n, j]) for n in range(_ND)], axis=1)
            r = jnp.dot(x, _load(wqbuf.at[ws, h]), preferred_element_type=f32)
            q[u] = (r * _QSCALE).astype(bf16)

        def qk(u):
            j, h = divmod(u, _HB)
            if h % (_HB // _CHUNKS[j]) == 0:
                wait(*kv_part(0, slot, j, h * _CHUNKS[j] // _HB, _CHUNKS[j]))
            scores[u] = lax.dot_general(q[u], _load(kvbuf.at[slot, j, 0, h]), _NT,
                                        preferred_element_type=f32)
            if h == _HB - 1:
                if j % 2 == 0:
                    @pl.when(i1 == _XB_AT)
                    def _():
                        for n in range(_ND):
                            start_x(1, j // 2, n)
                if j == 0:
                    for hh in range(_HB):
                        for_branch(more, br1, lambda s: start_wq(s, ws1, g1, hh))
                for c in range(_CHUNKS[j]):
                    for_branch(more, br1, lambda s: start_kv(s, 0, slot1, j, g1, c, _CHUNKS[j]))

        def softmax_pv(u):
            j, h = divmod(u, _HB)
            s = scores[u]
            e = jnp.exp2(s - jnp.max(s, axis=-1, keepdims=True))
            denom = jnp.sum(e, axis=-1, keepdims=True)
            if h % (_HB // _CHUNKS[j]) == 0:
                wait(*kv_part(1, slot, j, h * _CHUNKS[j] // _HB, _CHUNKS[j]))
            r = jnp.dot(e.astype(bf16), _load(kvbuf.at[slot, j, 1, h]), preferred_element_type=f32)
            r0 = pl.reciprocal(denom, approx=True)
            inv = r0 * (2.0 - denom * r0)
            obuf[j % 2, h] = (r * inv).astype(bf16)
            if h == _HB - 1:
                for c in range(_CHUNKS[j]):
                    for_branch(more, br1, lambda s_: start_kv(s_, 1, slot1, j, g1, c, _CHUNKS[j]))
                if j == 0:
                    for n in range(_ND):
                        for_branch(more, br1, lambda s_: start_wo(s_, ws1, g1, n))

        def out_proj(j, n):
            if j == 0 and n == 0:
                wait(wobuf.at[ws], swo.at[ws])
            o = jnp.concatenate([_load(obuf.at[j % 2, h]) for h in range(_HB)], axis=1)
            r = jnp.dot(o, _load(wobuf.at[ws, n]), preferred_element_type=f32)
            cols = slice(n * 128, (n + 1) * 128)
            r = r + acc[br, j, :, cols]
            acc[br, j, :, cols] = r
            ostage[br, j, n] = r.astype(bf16)

            @pl.when(g == _G - 1)
            def _():
                col = pl.multiple_of(br * _D + n * 128, 128)
                pltpu.make_async_copy(ostage.at[br, j, n], out.at[j, :, pl.ds(col, 128)],
                                      so.at[0]).start()

        for u in range(units):
            q_proj(u)
        for t in range(-1, units):
            if t + 1 < units:
                qk(t + 1)
            if t >= 0:
                j, h = divmod(t, _HB)
                if j >= 1:
                    for n in range(_ND):
                        if _OP_SLOT[n] == h:
                            out_proj(j - 1, n)
                softmax_pv(t)
        for n in range(_ND):
            out_proj(_B - 1, n)
        return ws1

    lax.fori_loop(0, _NP, phase, jnp.int32(0), unroll=2)
    wait(ostage, so.at[0])


@jax.jit
def pallas_concat_heads__mha_block_cached__mha_block_cached__near_ridge_kernel(
    A_x: jax.Array,
    A_k_cache: jax.Array,
    A_v_cache: jax.Array,
    A_wq: jax.Array,
    A_wo: jax.Array,
    B_x: jax.Array,
    B_k_cache: jax.Array,
    B_v_cache: jax.Array,
    B_wq: jax.Array,
    B_wo: jax.Array,
):
    bf16 = jnp.bfloat16
    hbm = pl.BlockSpec(memory_space=pl.ANY)
    dma = pltpu.SemaphoreType.DMA
    return pl.pallas_call(
        _kernel,
        in_specs=[hbm] * 10,
        out_specs=hbm,
        out_shape=jax.ShapeDtypeStruct((_B, _SQ, 2 * _D), bf16),
        scratch_shapes=[
            pltpu.VMEM((2, _B, 2, _HB, _SK, _DH), bf16),
            pltpu.VMEM((3, _HB, _D, _DH), bf16),
            pltpu.VMEM((3, _ND, _HB * _DH, 128), bf16),
            pltpu.VMEM((2, _ND, _B, _SQ, 128), bf16),
            pltpu.VMEM((2, _B, _SQ, _D), jnp.float32),
            pltpu.VMEM((2, _HB, _SQ, _DH), bf16),
            pltpu.VMEM((2, _B, _ND, _SQ, 128), bf16),
            dma((3, _B, 2 * _MC)), dma((3,)), dma((2, _B // 2)), dma((1,)),
        ],
        compiler_params=pltpu.CompilerParams(
            vmem_limit_bytes=100 * 1024 * 1024,
            disable_bounds_checks=True,
            disable_semaphore_checks=True,
            flags={"XLA_TPU_RESCHEDULE_DMA_DONES": True},
        ),
    )(A_x, A_k_cache, A_v_cache, A_wq, A_wo, B_x, B_k_cache, B_v_cache, B_wq, B_wo)
```

```python
import jax
import jax.numpy as jnp
from jax import lax
import jax.experimental.pallas as pl
import jax.experimental.pallas.tpu as pltpu

_B, _SQ, _D = 8, 144, 640
_H, _SK, _DH = 32, 512, 128
_HB = 4
_G = _H // _HB
_LG = 3
_NP = 2 * _G
_ND = _D // 128
_OP_SLOT = (0, 0, 1, 1, 2)
_CHUNKS = (1, 1, 1, 1, 2, 2, 2, 2)
_NPLAIN = 4
_MC = 2
_XB_AT = 5
_QSCALE = (_DH ** -0.5) * 1.4426950408889634
_NT = (((1,), (1,)), ((), ()))


def _loop(lo, hi, fn):
    def step(t, carry):
        fn(t)
        return carry
    lax.fori_loop(lo, hi, step, 0)


def _kernel(ax, ak, av, awq, awo, bx, bk, bv, bwq, bwo, out,
            kvbuf, wqbuf, wobuf, xbuf, acc, obuf, ostage, skv, swo, sx, so):
    f32, bf16 = jnp.float32, jnp.bfloat16
    x_hbm, wq_hbm, wo_hbm = (ax, bx), (awq, bwq), (awo, bwo)
    kv_hbm = ((ak, bk), (av, bv))

    def wait(dst, sem):
        pltpu.make_async_copy(dst, dst, sem).wait()

    def for_branch(pred, br, fn):
        pl.when(jnp.logical_and(pred, br == 0))(lambda: fn(0))
        pl.when(jnp.logical_and(pred, br == 1))(lambda: fn(1))

    def kv_part(w, slot, j, c, chunks):
        n = _HB // chunks
        return kvbuf.at[slot, j, w, pl.ds(c * n, n)], skv.at[slot, j, w * _MC + c]

    def start_kv(s, w, slot, j, g, c=0, chunks=1):
        n = _HB // chunks
        pltpu.make_async_copy(kv_hbm[w][s].at[j, pl.ds(g * _HB + c * n, n)],
                              *kv_part(w, slot, j, c, chunks)).start()

    def start_wq(s, ws, g, h):
        col = pl.multiple_of((g * _HB + h) * _DH, _DH)
        pltpu.make_async_copy(wq_hbm[s].at[:, pl.ds(col, _DH)],
                              wqbuf.at[ws, h], skv.at[2, ws, 0]).start()

    def start_wo(s, ws, g, n):
        row = pl.multiple_of(g * (_HB * _DH), _HB * _DH)
        pltpu.make_async_copy(wo_hbm[s].at[pl.ds(row, _HB * _DH), pl.ds(n * 128, 128)],
                              wobuf.at[ws, n], swo.at[ws]).start()

    def start_x(s, pair, n):
        col = pl.multiple_of(n * 128, 128)
        pltpu.make_async_copy(x_hbm[s].at[pl.ds(2 * pair, 2), :, pl.ds(col, 128)],
                              xbuf.at[s, n, pl.ds(2 * pair, 2)], sx.at[s, pair]).start()

    _loop(0, _ND, lambda n: start_x(0, 0, n))
    _loop(0, _HB, lambda h: start_wq(0, 0, 0, h))

    def request_x_pair(pair):
        for n in range(_ND):
            start_x(0, pair, n)
    _loop(1, _B // 2, request_x_pair)
    _loop(0, _HB, lambda h: start_wq(0, 1, 1, h))

    def request_first_kv(j):
        @pl.when(j == 1)
        def _():
            for n in range(_ND):
                start_wo(0, 0, 0, n)
        start_kv(0, 0, 0, j, 0)
        start_kv(0, 1, 0, j, 0)
    _loop(0, _NPLAIN, request_first_kv)
    for j in range(_NPLAIN, _B):
        for c in range(_CHUNKS[j]):
            start_kv(0, 0, 0, j, 0, c, _CHUNKS[j])
            start_kv(0, 1, 0, j, 0, c, _CHUNKS[j])

    acc[...] = jnp.zeros(acc.shape, f32)

    def phase(i):
        g, br, slot, ws = i & (_G - 1), i >> _LG, i & 1, i & 3
        i1, i2 = i + 1, i + 2
        g1, br1, slot1, ws1 = i1 & (_G - 1), i1 >> _LG, i1 & 1, i1 & 3
        g2, br2, ws2 = i2 & (_G - 1), i2 >> _LG, i2 & 3
        more, more2 = i1 < _NP, i2 < _NP
        units = _B * _HB
        q, scores = {}, {}

        def q_proj(u):
            j, h = divmod(u, _HB)
            if h == 0 and j % 2 == 0:
                pl.when(g == 0)(lambda: wait(xbuf.at[br, :, pl.ds(j, 2)], sx.at[br, j // 2]))
            if u == 0:
                wait(wqbuf.at[ws], skv.at[2, ws, 0])
            x = jnp.concatenate([xbuf[br, n, j] for n in range(_ND)], axis=1)
            r = jnp.dot(x, wqbuf[ws, h], preferred_element_type=f32)
            q[u] = (r * _QSCALE).astype(bf16)

        def qk(u):
            j, h = divmod(u, _HB)
            if h % (_HB // _CHUNKS[j]) == 0:
                wait(*kv_part(0, slot, j, h * _CHUNKS[j] // _HB, _CHUNKS[j]))
            scores[u] = lax.dot_general(q[u], kvbuf[slot, j, 0, h], _NT,
                                        preferred_element_type=f32)
            if h == _HB - 1:
                if j % 2 == 0:
                    @pl.when(i1 == _XB_AT)
                    def _():
                        for n in range(_ND):
                            start_x(1, j // 2, n)
                if j == 0:
                    for hh in range(_HB):
                        for_branch(more2, br2, lambda s: start_wq(s, ws2, g2, hh))
                for c in range(_CHUNKS[j]):
                    for_branch(more, br1, lambda s: start_kv(s, 0, slot1, j, g1, c, _CHUNKS[j]))

        def softmax_pv(u):
            j, h = divmod(u, _HB)
            s = scores[u]
            e = jnp.exp2(s - jnp.max(s, axis=-1, keepdims=True))
            denom = jnp.sum(e, axis=-1, keepdims=True)
            if h % (_HB // _CHUNKS[j]) == 0:
                wait(*kv_part(1, slot, j, h * _CHUNKS[j] // _HB, _CHUNKS[j]))
            r = jnp.dot(e.astype(bf16), kvbuf[slot, j, 1, h], preferred_element_type=f32)
            r0 = pl.reciprocal(denom, approx=True)
            inv = r0 * (2.0 - denom * r0)
            obuf[j % 2, h] = pltpu.bitcast((r * inv).astype(bf16), jnp.uint32)
            if h == _HB - 1:
                for c in range(_CHUNKS[j]):
                    for_branch(more, br1, lambda s_: start_kv(s_, 1, slot1, j, g1, c, _CHUNKS[j]))
                if j == 0:
                    for n in range(_ND):
                        for_branch(more, br1, lambda s_: start_wo(s_, ws1, g1, n))

        def out_proj(j, n):
            if j == 0 and n == 0:
                wait(wobuf.at[ws], swo.at[ws])
            o = jnp.concatenate([pltpu.bitcast(obuf[j % 2, h], bf16) for h in range(_HB)], axis=1)
            r = jnp.dot(o, wobuf[ws, n], preferred_element_type=f32)
            cols = slice(n * 128, (n + 1) * 128)
            r = r + acc[br, j, :, cols]
            acc[br, j, :, cols] = r
            ostage[br, j, n] = r.astype(bf16)

            @pl.when(g == _G - 1)
            def _():
                col = pl.multiple_of(br * _D + n * 128, 128)
                pltpu.make_async_copy(ostage.at[br, j, n], out.at[j, :, pl.ds(col, 128)],
                                      so.at[0]).start()

        def project_q():
            for u in range(units):
                q_proj(u)

        def attend():
            for t in range(-1, units):
                if t + 1 < units:
                    qk(t + 1)
                if t >= 0:
                    j, h = divmod(t, _HB)
                    if j >= 1:
                        for n in range(_ND):
                            if _OP_SLOT[n] == h:
                                out_proj(j - 1, n)
                    softmax_pv(t)
            for n in range(_ND):
                out_proj(_B - 1, n)
        return project_q, attend

    def trip(t):
        project_a, attend_a = phase(2 * t)
        project_b, attend_b = phase(2 * t + 1)
        project_a()
        project_b()
        attend_a()
        attend_b()

    _loop(0, _NP // 2, trip)
    wait(ostage, so.at[0])


@jax.jit
def pallas_concat_heads__mha_block_cached__mha_block_cached__near_ridge_kernel(
    A_x: jax.Array,
    A_k_cache: jax.Array,
    A_v_cache: jax.Array,
    A_wq: jax.Array,
    A_wo: jax.Array,
    B_x: jax.Array,
    B_k_cache: jax.Array,
    B_v_cache: jax.Array,
    B_wq: jax.Array,
    B_wo: jax.Array,
):
    bf16 = jnp.bfloat16
    hbm = pl.BlockSpec(memory_space=pl.ANY)
    dma = pltpu.SemaphoreType.DMA
    return pl.pallas_call(
        _kernel,
        in_specs=[hbm] * 10,
        out_specs=hbm,
        out_shape=jax.ShapeDtypeStruct((_B, _SQ, 2 * _D), bf16),
        scratch_shapes=[
            pltpu.VMEM((2, _B, 2, _HB, _SK, _DH), bf16),
            pltpu.VMEM((4, _HB, _D, _DH), bf16),
            pltpu.VMEM((4, _ND, _HB * _DH, 128), bf16),
            pltpu.VMEM((2, _ND, _B, _SQ, 128), bf16),
            pltpu.VMEM((2, _B, _SQ, _D), jnp.float32),
            pltpu.VMEM((2, _HB, _SQ // 2, _DH), jnp.uint32),
            pltpu.VMEM((2, _B, _ND, _SQ, 128), bf16),
            dma((3, _B, 2 * _MC)), dma((4,)), dma((2, _B // 2)), dma((1,)),
        ],
        compiler_params=pltpu.CompilerParams(
            vmem_limit_bytes=100 * 1024 * 1024,
            disable_bounds_checks=True,
            disable_semaphore_checks=True,
            flags={"XLA_TPU_RESCHEDULE_DMA_DONES": True},
        ),
    )(A_x, A_k_cache, A_v_cache, A_wq, A_wo, B_x, B_k_cache, B_v_cache, B_wq, B_wo)
```
